```python
import jax
import jax.numpy as jnp

def _softmax(x, axis=-1):
    return jax.nn.softmax(x, axis=axis)
def _gelu(x):
    return jax.nn.gelu(x, approximate=True)
def _silu(x):
    return jax.nn.silu(x)
def _sigmoid(x):
    return jax.nn.sigmoid(x)
def _layernorm(x, axis=-1, eps=1e-5):
    m = jnp.mean(x, axis=axis, keepdims=True)
    v = jnp.var(x, axis=axis, keepdims=True)
    return (x - m) / jnp.sqrt(v + eps)
def _scatter_add(tgt, idx, src, axis=0):
    return tgt.at[idx].add(src)
def _segment_sum(src, seg, n):
    return jax.ops.segment_sum(src, seg, n)
class _Rng:
    def __init__(self, key):
        self._k = key
    def _next(self):
        self._k, sub = jax.random.split(self._k)
        return sub
    def normal(self, shape):
        return jax.random.normal(self._next(), shape, dtype=jnp.bfloat16)
    def randint(self, lo, hi, shape):
        return jax.random.randint(self._next(), shape, lo, hi, dtype=jnp.int32)
    def uniform(self, shape, lo=0.0, hi=1.0):
        return jax.random.uniform(self._next(), shape, jnp.bfloat16, lo, hi)
    def permutation(self, n):
        return jax.random.permutation(self._next(), n)


kernel_name = 'concat_heads__ssm_conv_h3__softmax_full_mha__prompt'

def _fwd_setup_inputs():
    _rng = _Rng(jax.random.key(int.from_bytes(__import__("os").urandom(4), "little")))
    _w = (lambda a: (lambda t: t.astype(jnp.bfloat16) if jnp.issubdtype(t.dtype, jnp.floating) else t)(jnp.asarray(a)))
    def _A_setup():
        B, S, D = 1, 2048, 640
        ks = 4
        return {
            "q": _w((lambda *s: _rng.normal(s) * 0.05)(B, S, D)),
            "k": _w((lambda *s: _rng.normal(s) * 0.05)(B, S, D)),
            "v": _w((lambda *s: _rng.normal(s) * 0.05)(B, S, D)),
            "shift_k": _w((lambda *s: _rng.normal(s) * 0.05)(D, ks) * 0.5),
            "ssm_k": _w((lambda *s: _rng.normal(s) * 0.05)(D, S) * (1.0 / S ** 0.5)),
            "ssm_D": _w((lambda *s: _rng.normal(s) * 0.05)(D)),
        }
    _A_in = _A_setup()

    def _B_setup():
        B, S, D = 1, 2048, 640
        return {
            "x": _w((lambda *s: _rng.normal(s) * 0.05)(B, S, D)),
            "wqkv": _w((lambda *s: _rng.normal(s) * 0.05)(D, 3 * D)),
            "wo": _w((lambda *s: _rng.normal(s) * 0.05)(D, D)),
        }
    _B_in = _B_setup()

    return {
        "A_q": _A_in["q"],
        "A_k": _A_in["k"],
        "A_v": _A_in["v"],
        "A_shift_k": _A_in["shift_k"],
        "A_ssm_k": _A_in["ssm_k"],
        "A_ssm_D": _A_in["ssm_D"],
        "B_x": _B_in["x"],
        "B_wqkv": _B_in["wqkv"],
        "B_wo": _B_in["wo"],
    }

def _fwd_reference(A_q, A_k, A_v, A_shift_k, A_ssm_k, A_ssm_D, B_x, B_wqkv, B_wo):
    def _A_ref(q, k, v, shift_k, ssm_k, ssm_D):
        B, S, D = q.shape
        ks = shift_k.shape[-1]
        k_pad = jnp.pad(k, ((0, 0), (ks - 1, 0), (0, 0)))
        k_shift = jnp.zeros_like(k)
        for t in range(ks):
            k_shift = k_shift + k_pad[:, t:t + S, :] * shift_k[:, ks - 1 - t][None, None, :]
        kv = k_shift * v
        L = 2 * S
        kv_pad = jnp.pad(kv, ((0, 0), (0, S), (0, 0)))
        kf_pad = jnp.pad(ssm_k, ((0, 0), (0, S)))
        kv_f = (lambda x, axes=(-2,-1): jnp.fft.rfft2(x.astype(jnp.float32), axes=axes))(kv_pad[:, None, :, :], axes=(1, 2))
        kf_f = (lambda x, axes=(-2,-1): jnp.fft.rfft2(x.astype(jnp.float32), axes=axes))(kf_pad[:, None, :], axes=(1, 2))
        kf_f = (lambda x, *d: x.transpose(*d))(kf_f, 1, 2, 0)
        y_f = kv_f * kf_f[None, :, :, :]
        y = (lambda x, s, axes=(-2,-1): jnp.fft.irfft2(x, s=s, axes=axes).astype(jnp.bfloat16))(y_f, (1, L), axes=(1, 2))[:, 0, :S, :]
        y = y + kv * ssm_D[None, None, :]
        return q * y

    def _B_ref(x, wqkv, wo):
        B, S, D = x.shape
        H = 32; Dh = D // H
        qkv = (lambda x, *d: x.transpose(*d))((x @ wqkv).reshape(B, S, 3, H, Dh), 2, 0, 3, 1, 4)
        q, k, v = qkv[0], qkv[1], qkv[2]
        scale = Dh ** -0.5
        scores = jnp.einsum("bhqd,bhkd->bhqk", q, k) * scale
        p = _softmax(scores, axis=-1)
        o = jnp.einsum("bhqk,bhkd->bhqd", p, v)
        return (lambda x, *d: x.transpose(*d))(o, 0, 2, 1, 3).reshape(B, S, D) @ wo

    a = _A_ref(A_q, A_k, A_v, A_shift_k, A_ssm_k, A_ssm_D)
    b = _B_ref(B_x, B_wqkv, B_wo)
    return jnp.concatenate([a, b], axis=-1)


def setup_inputs():
    _inp = _fwd_setup_inputs()
    _gk = jax.random.fold_in(jax.random.key(int.from_bytes(__import__("os").urandom(4), "little")), 2**31 - 1)
    _shapes = [[1, 2048, 1280]]
    _dtypes = ['bfloat16']
    _gks = jax.random.split(_gk, len(_shapes))
    _gs = [jax.random.normal(k, s, dtype=jnp.dtype(d)) * 0.05 for k, s, d in zip(_gks, _shapes, _dtypes)]
    _inp["grad_out"] = _gs[0]
    return _inp

def reference(A_q, A_k, A_v, A_shift_k, A_ssm_k, A_ssm_D, B_x, B_wqkv, B_wo, grad_out):
    _const = dict()
    def _f(*_d):
        return _fwd_reference(**{'A_q': _d[0], 'A_k': _d[1], 'A_v': _d[2], 'A_shift_k': _d[3], 'A_ssm_k': _d[4], 'A_ssm_D': _d[5], 'B_x': _d[6], 'B_wqkv': _d[7], 'B_wo': _d[8], **_const})
    _out, _vjp = jax.vjp(_f, A_q, A_k, A_v, A_shift_k, A_ssm_k, A_ssm_D, B_x, B_wqkv, B_wo)
    _grads = _vjp(grad_out)
    _out0 = jnp.asarray(_out)
    return (_out0, *[jnp.asarray(_g) for _g in _grads])
```

```python
import math

import numpy as np
import jax
import jax.numpy as jnp
from jax import lax
import jax.experimental.pallas as pl
import jax.experimental.pallas.tpu as pltpu

f32 = jnp.float32
bf16 = jnp.bfloat16

S = 2048
D = 640
NH = 32
DH = 20
NP = 16
G = 40
M = 24
TQ = 512
TK = 256
NQ = S // TQ
LOG_NQ = NQ.bit_length() - 1
NC = S // TK
NIT = NP * NQ
KS_W = 32
KP_W = 48
R0 = (0, G - M)
V0 = (0, M - DH)
SP0 = (DH, 0)
UNR = 2
CB = 128
NB = S // CB
NF = 2 * CB
NPOS = CB // 8
NG = D // 128
UPG = 3 * NPOS
IPG = UPG // 4
PPG = IPG // NQ
SCALE = DH ** -0.5
LOG2E = math.log2(math.e)
LN2 = math.log(2.0)
SAFE_BOUND = 24.0

NN = (((1,), (0,)), ((), ()))
NT = (((1,), (1,)), ((), ()))

SEM_GB = 0
SEM_W, SEM_X, SEM_CONV, SEM_OUT = 5, 6, 7, 8
NSEM = 9
GB_CHUNKS = ((0, 256), (256, 256), (512, 512), (1024, 512), (1536, 512))


PLAN = tuple(
    (((0, NB - 1 - c),), ((1, NB // 2 - 1 - c),), ((0, c),), (), ((1, NB // 2 + c),), ())
    for c in range(NC))


def _dg(a, b, dn):
    return lax.dot_general(a, b, dn, preferred_element_type=f32)


def _dft_mats():
    f = np.concatenate([np.arange(0, CB, 2), np.arange(1, CB, 2)]).astype(np.float64)
    n = np.arange(CB, dtype=np.float64)
    th = 2.0 * np.pi * (f[:, None] + 0.5) * n[None, :] / (2 * CB)

    def rows(re, im):
        return np.stack([re.reshape(NPOS, 8, CB), im.reshape(NPOS, 8, CB)], axis=1).reshape(NF, CB)

    fwd = rows(np.cos(th), -np.sin(th))
    fwdc = rows(np.cos(th), np.sin(th))
    fw = np.stack([fwd, fwdc])
    fi = np.stack([fwd.T / CB, fwdc.T / CB])
    return fw.astype(np.float32), fi.astype(np.float32)


def _fill_spare(win, par, b):
    b = -b
    h = b.astype(bf16).astype(f32)
    r = b - h
    m = r.astype(bf16).astype(f32)
    l = (r - m).astype(bf16).astype(f32)
    row = lax.broadcasted_iota(jnp.int32, win.shape, 0)
    s0 = SP0[par]
    return jnp.where(row == s0, h, jnp.where(row == s0 + 1, m, jnp.where(
        row == s0 + 2, l, jnp.where(row == s0 + 3, 0.0, win))))


def _spare_mask(shape, par):
    row = lax.broadcasted_iota(jnp.int32, shape, 0)
    return (row >= DH) if par == 0 else (row < M - DH)


def _shift_add(cur, prev):
    h = NPOS // 2
    cr, ci, pr, pi = cur[:, 0:8], cur[:, 8:16], prev[:, 0:8], prev[:, 8:16]
    re = jnp.concatenate([cr[:h] - pi[:h], cr[h:] + pi[h:]], axis=0)
    im = jnp.concatenate([ci[:h] + pr[:h], ci[h:] - pr[h:]], axis=0)
    return jnp.concatenate([re, im], axis=1)


def _kernel(q_hbm, k_hbm, v_hbm, sk_hbm, hk_hbm, dd_hbm, x_hbm, wqkv_hbm, wo_hbm, g_hbm,
            fw_hbm, fi_hbm,
            out_hbm, dq_hbm, dk_hbm, dv_hbm, dsk_hbm, dhk_hbm, ddd_hbm, dx_hbm, dwqkv_hbm, dwo_hbm,
            q_v, k_v, v_v, ga_v, hk_v, x_v, gb_v, wqkv_v, wo_v,
            wt_s, qkvt, dqkvt, dot_s, kva, b_s, p_a, p_b, qw_c, oa_c, ds_c, dq_c,
            dqkvb, ob_s, xt_s, dwqkv_s, dwo_s,
            ks_s, spec, res, fw_ref, fi_ref, dd_s, sk_ref, dsk_ref, dd1, ddd1,
            sems):
    def cp(src, dst, i):
        return pltpu.make_async_copy(src, dst, sems.at[i])

    XC = 512

    def rows_of(c):
        return pl.ds(pl.multiple_of(c * XC, XC), XC)

    def lanes_of(g):
        return pl.ds(pl.multiple_of(g * 128, 128), 128)

    def conv_in(g):
        return [cp(src.at[0, :, lanes_of(g)], dst.at[g], SEM_CONV)
                for src, dst in ((k_hbm, k_v), (v_hbm, v_v), (q_hbm, q_v), (g_hbm, ga_v))]

    def conv_out(g):
        cs = [cp(src.at[g], dst.at[0, :, lanes_of(g)], SEM_OUT)
              for src, dst in ((k_v, dk_hbm), (v_v, dv_hbm), (q_v, dq_hbm), (ga_v, out_hbm))]
        cs.append(cp(hk_v.at[lanes_of(g), :], dhk_hbm.at[lanes_of(g), :], SEM_OUT))
        return cs

    c_w = cp(wqkv_hbm, wqkv_v, SEM_W)
    c_wo = cp(wo_hbm, wo_v, SEM_GB)
    c_x = cp(x_hbm.at[0], x_v, SEM_X)
    c_gb = [cp(g_hbm.at[0, pl.ds(r0, nr), pl.ds(D, D)], gb_v.at[pl.ds(r0, nr), :], SEM_GB + j)
            for j, (r0, nr) in enumerate(GB_CHUNKS)]
    c_conv = [cp(hk_hbm, hk_v, SEM_CONV), cp(fw_hbm, fw_ref, SEM_CONV), cp(fi_hbm, fi_ref, SEM_CONV),
              cp(sk_hbm, sk_ref, SEM_CONV), cp(dd_hbm, dd1, SEM_CONV)]
    for g in range(NG):
        c_conv += conv_in(g)
    c_dsk = cp(dsk_ref, dsk_hbm, SEM_OUT)
    c_ddd = cp(ddd1, ddd_hbm, SEM_OUT)

    TD = 256
    NDA = 5

    for c in [c_wo] + c_gb[:-1] + [c_w, c_gb[-1], c_x] + c_conv:
        c.start()
    c_wo.wait()
    c_gb[0].wait()

    def dot_chunk(n, waits):
        for j in waits:
            @pl.when(n == GB_CHUNKS[j][0] // TD)
            def _():
                c_gb[j].wait()

        cols = pl.ds(pl.multiple_of(n * TD, TD), TD)
        r = _dg(wo_v[...], gb_v[cols, :], NT)
        dot_s[:, :, cols] = r.reshape(NP, G, TD)

    def dot_body_a(n, carry):
        dot_chunk(n, (1, 2, 3))
        return carry

    def dot_body_b(n, carry):
        dot_chunk(n + NDA, (4,))
        wc = pl.ds(pl.multiple_of(n * D, 128), D)
        wt_s[wc, :] = wqkv_v[:, wc].T
        return carry

    lax.fori_loop(0, NDA, dot_body_a, 0)
    c_w.wait()
    lax.fori_loop(0, S // TD - NDA, dot_body_b, 0)
    c_x.wait()

    def amax8(a):
        return jnp.max(jnp.abs(a).reshape(D // 8, 8, XC), axis=0)

    def proj_body(n, carry):
        cols = rows_of(n)
        xc = x_v[cols, :]
        xt_s[:, cols] = xc.T
        kt = _dg(wt_s[D:2 * D, :], xc, NT)
        qkvt[NP:2 * NP, :, cols] = kt.reshape(NP, G, XC)
        vt = _dg(wt_s[2 * D:3 * D, :], xc, NT)
        qkvt[2 * NP:3 * NP, :, cols] = vt.reshape(NP, G, XC)
        for h in range(NH):
            r0 = (h // 2) * G + R0[h % 2]
            kw = jnp.where(_spare_mask((M, XC), h % 2), 1.0, kt[r0:r0 + M])
            t = jnp.concatenate([kw, vt[r0:r0 + M], jnp.zeros((128 - 2 * M, XC), f32)], axis=0)
            kva[h, cols, :] = t.T.astype(bf16)
        qt = _dg(wt_s[0:D, :], xc, NT) * (SCALE * LOG2E)
        qkvt[0:NP, :, cols] = qt.reshape(NP, G, XC)
        return jnp.maximum(carry[0], amax8(qt)), jnp.maximum(carry[1], amax8(kt))

    qm, km = lax.fori_loop(0, S // XC, proj_body, (jnp.zeros((8, XC), f32), jnp.zeros((8, XC), f32)))

    def allmax(a):
        return jnp.max(jnp.max(a, axis=1, keepdims=True), axis=0, keepdims=True)

    bound = allmax(qm) * allmax(km) * (DH * 1.02)
    b_s[...] = jnp.broadcast_to(bound, b_s.shape)
    unsafe = jnp.logical_not(jnp.max(bound) <= SAFE_BOUND)

    def q_weights(i, par, off, b):
        qt = _fill_spare(qkvt[i, R0[par]:R0[par] + M, pl.ds(off, TQ)], par, b)
        return jnp.concatenate([qt, jnp.zeros((KS_W - M, TQ), f32)], axis=0).astype(bf16)

    @pl.when(unsafe)
    def _():
        def mx_body(t, carry):
            i = t // NQ
            off = pl.multiple_of((t % NQ) * TQ, TQ)
            for par in range(2):
                qw = q_weights(i, par, off, jnp.zeros((1, TQ), f32))

                def mx_chunk(c, m):
                    ro = pl.multiple_of(c * TK, TK)
                    s = _dg(kva[2 * i + par, pl.ds(ro, TK), :KS_W], qw, NN)
                    return jnp.maximum(m, jnp.max(s, axis=0, keepdims=True))

                m = lax.fori_loop(0, NC, mx_chunk, jnp.full((1, TQ), -jnp.inf, f32))
                b_s[pl.ds(2 * i + par, 1), pl.ds(off, TQ)] = m
            return carry
        lax.fori_loop(0, NIT, mx_body, 0)

    for c in c_conv:
        c.wait()
    dd_s[0:1, :] = dd1[...].astype(f32).reshape(1, D)

    def blk(a):
        return slice(16 * a, 16 * a + 16)

    def taps(g):
        w4 = sk_ref[:, lanes_of(g)].astype(f32)
        return [w4[j:j + 1, :] for j in range(4)]

    def conv_pre(g):
        L = lanes_of(g)
        wj = taps(g)
        yp = None
        tail = jnp.zeros((8, 128), f32)
        for a in range(NB):
            r0 = a * CB
            rows = slice(r0, r0 + CB)
            kf = k_v[g, rows, :].astype(f32)
            ext = jnp.concatenate([tail, kf], axis=0)
            tail = kf[CB - 8:CB]
            ks = kf * wj[0]
            for j in range(1, 4):
                ks = ks + pltpu.roll(ext, j, 0)[8:8 + CB] * wj[j]
            ks_s[rows, :] = ks
            kv = ks * v_v[g, rows, :].astype(f32)
            dy = ga_v[g, rows, :].astype(f32) * q_v[g, rows, :].astype(f32)
            h = _dg(fw_ref[0], hk_v[L, rows], NT).reshape(NPOS, 16, 128)
            if a == 0:
                dvec = dd_s[0:1, L]
                h = jnp.concatenate([h[:, 0:8] + dvec[None], h[:, 8:16]], axis=1)
            spec[0, :, blk(a), :] = h
            spec[1, :, blk(a), :] = _dg(fw_ref[0], kv.astype(bf16), NN).reshape(NPOS, 16, 128)
            y = _dg(fw_ref[1], dy.astype(bf16), NN).reshape(NPOS, 16, 128)
            if yp is not None:
                spec[2, :, blk(NB - a), :] = _shift_add(yp, y)
            if a == NB - 1:
                spec[2, :, blk(0), :] = y
            yp = y

    def conv_mac(u):
        u = lax.rem(jnp.minimum(u, NG * UPG - 1), UPG)
        kind = lax.shift_right_logical(u, NPOS.bit_length() - 1)
        pos = u & (NPOS - 1)
        ia = lax.shift_right_logical(kind, 1)
        ib = 1 + jnp.minimum(kind, 1)

        def re(a):
            return slice(16 * a, 16 * a + 8)

        def im(a):
            return slice(16 * a + 8, 16 * a + 16)

        def emit(a):
            zr = zi = None
            for b in range(a + 1):
                ar, ai = spec[ia, pos, re(b), :], spec[ia, pos, im(b), :]
                br, bi = spec[ib, pos, re(a - b), :], spec[ib, pos, im(a - b), :]
                tr = ar * br - ai * bi
                ti = ar * bi + ai * br
                zr = tr if zr is None else zr + tr
                zi = ti if zi is None else zi + ti
            res[kind, pos, re(a), :] = zr
            res[kind, pos, im(a), :] = zi

        return emit

    def conv_post(g):
        L = lanes_of(g)
        wj = taps(g)
        acc = [jnp.zeros((8, 128), f32) for _ in range(4)]
        head = jnp.zeros((8, 128), f32)
        for a in range(NB - 1, -1, -1):
            r0 = a * CB
            rows = slice(r0, r0 + CB)
            z = res[0, :, blk(a), :]
            if a > 0:
                z = _shift_add(z, res[0, :, blk(a - 1), :])
            dh = _dg(fi_ref[1], res[2, :, blk(NB - 1 - a), :].reshape(NF, 128), NN)
            dkv = _dg(fi_ref[1], res[1, :, blk(NB - 1 - a), :].reshape(NF, 128), NN)
            y = _dg(fi_ref[0], z.reshape(NF, 128), NN)
            hk_v[L, rows] = dh.T.astype(bf16)
            if a == 0:
                dd_s[1:2, L] = dh[0:1, :]
            dks = dkv * v_v[g, rows, :].astype(f32)
            v_v[g, rows, :] = (dkv * ks_s[rows, :]).astype(bf16)
            ext = jnp.concatenate([dks, head], axis=0)
            head = dks[0:8]
            kf = k_v[g, rows, :].astype(f32)
            dk = None
            for j in range(4):
                dj = dks if j == 0 else pltpu.roll(ext, CB + 8 - j, 0)[0:CB]
                dk = dj * wj[j] if dk is None else dk + dj * wj[j]
                acc[j] = acc[j] + jnp.sum((dj * kf).reshape(CB // 8, 8, 128), axis=0)
            k_v[g, rows, :] = dk.astype(bf16)
            qf = q_v[g, rows, :].astype(f32)
            gf = ga_v[g, rows, :].astype(f32)
            ga_v[g, rows, :] = (qf * y).astype(bf16)
            q_v[g, rows, :] = (gf * y).astype(bf16)
        row = lax.broadcasted_iota(jnp.int32, (4, 128), 0)
        r4 = jnp.zeros((4, 128), f32)
        for j in range(4):
            r4 = jnp.where(row == j, jnp.sum(acc[j], axis=0, keepdims=True), r4)
        dsk_ref[:, L] = r4.astype(bf16)
        for c in conv_out(g):
            c.start()

    P = [p_a, p_b]

    def item(t):
        if isinstance(t, int):
            return t // NQ, (t % NQ) * TQ
        return lax.shift_right_logical(t, LOG_NQ), pl.multiple_of((t & (NQ - 1)) * TQ, TQ)

    def make_qw(t, par):
        i, off = item(t)
        return q_weights(i, par, off, b_s[pl.ds(2 * i + par, 1), pl.ds(off, TQ)])

    def finish1(t, par, oa):
        i, off = item(t)
        lo, hi = V0[par], V0[par] + DH
        do = dot_s[i, R0[par]:R0[par] + M, pl.ds(off, TQ)]
        r = 1.0 / oa[SP0[par]:SP0[par] + 1, :]
        o = oa * r
        dop = jnp.where(_spare_mask((M, TQ), par), 0.0, (do * r).astype(bf16).astype(f32))
        dot_s[i, par * DH:(par + 1) * DH, pl.ds(off, TQ)] = o[lo:hi]
        delta = jnp.sum(dop * o, axis=0, keepdims=True)
        top = _fill_spare(jnp.zeros((M, TQ), f32), par, delta)
        return jnp.concatenate([top, dop], axis=0).astype(bf16), dop

    def accum(t, idx, par, ck, val):
        dst = dqkvt.at[idx, par * DH:(par + 1) * DH, ck]
        dst[...] = jnp.where((t & (NQ - 1)) == 0, 0.0, dst[...]) + val

    def dkq(t, par, c, ds, dq, mid=None):
        i, off = item(t)
        lo, hi = V0[par], V0[par] + DH
        ck = slice(c * TK, (c + 1) * TK)
        qt = qkvt[i, R0[par]:R0[par] + M, pl.ds(off, TQ)] * LN2
        dk = _dg(qt, ds, NT)
        accum(t, NP + i, par, ck, dk[lo:hi])
        if mid is not None:
            mid()
        t_ = _dg(qkvt[NP + i, R0[par]:R0[par] + M, ck], ds, NN)
        dq = t_ if dq is None else t_ + dq
        if c == NC - 1:
            dqkvt[i, par * DH:(par + 1) * DH, pl.ds(off, TQ)] = (dq * SCALE)[lo:hi]
        return dq

    def scores(i, par, c, qw):
        s = _dg(kva[2 * i + par, c * TK:(c + 1) * TK, :KS_W], qw, NN)
        p = jnp.exp2(s).astype(bf16)
        P[par][c * TK // 2:(c + 1) * TK // 2, :] = pltpu.bitcast(p, jnp.uint32)
        return p

    def pv(i, par, c, p, oa):
        vt = qkvt[2 * NP + i, R0[par]:R0[par] + M, c * TK:(c + 1) * TK]
        vt = jnp.where(_spare_mask((M, TK), par), 1.0, vt)
        t_ = _dg(vt, p, NN)
        return t_ if oa is None else t_ + oa

    def step(t1, par1, t2, t3, qw, oa2, ds3, dq3, macs):
        par2 = 1 - par1
        i1, _ = item(t1)
        i2, _ = item(t2)
        lo2, hi2 = V0[par2], V0[par2] + DH
        oa = dq = ds = None
        for c in range(NC):
            def fill(slot):
                for k, a in PLAN[c][slot]:
                    macs[k](a)

            ck = slice(c * TK, (c + 1) * TK)
            p1 = scores(i1, par1, c, qw)
            fill(0)
            if c == 0:
                doa, dop = finish1(t2, par2, oa2)
                dkq(t3, par1, NC - 1, ds3, dq3, lambda: fill(1))
            else:
                dq = dkq(t2, par2, c - 1, ds, dq, lambda: fill(1))
            fill(2)
            p2 = pltpu.bitcast(P[par2][c * TK // 2:(c + 1) * TK // 2, :], bf16)
            dp = _dg(kva[2 * i2 + par2, ck, :KP_W], doa, NN)
            ds = (p2.astype(f32) * dp).astype(bf16)
            fill(3)
            dv = _dg(dop, p2, NT)
            accum(t2, 2 * NP + i2, par2, ck, dv[lo2:hi2])
            fill(4)
            oa = pv(i1, par1, c, p1, oa)
            fill(5)
        return oa, ds, dq

    qw0 = make_qw(0, 0)
    oa0 = None
    pprev = None
    for c in range(NC + 1):
        pcur = scores(0, 0, c, qw0) if c < NC else None
        if c > 0:
            oa0 = pv(0, 0, c - 1, pprev, oa0)
        pprev = pcur
    oa_c[...] = oa0
    qw_c[...] = make_qw(0, 1)

    def attn_body(tt, carry):
        @pl.when(tt == 0)
        def _():
            ds_c[...] = jnp.zeros(ds_c.shape, jnp.uint32)
            dq_c[...] = jnp.zeros(dq_c.shape, f32)

        qw_a, oa, dq = qw_c[...], oa_c[...], dq_c[...]
        ds = pltpu.bitcast(ds_c[...], bf16)
        for k in range(UNR):
            t = tt * UNR + k
            tp = jnp.maximum(t - 1, 0)
            tn = jnp.minimum(t + 1, NIT - 1)
            qw_b = make_qw(tn, 0)
            oa, ds, dq = step(t, 1, t, tp, qw_a, oa, ds, dq,
                              [conv_mac(4 * t), conv_mac(4 * t + 1)])
            qw_a = make_qw(tn, 1)
            if k == UNR - 1:
                qw_c[...] = qw_a
            oa, ds, dq = step(tn, 0, t, t, qw_b, oa, ds, dq,
                              [conv_mac(4 * t + 2), conv_mac(4 * t + 3)])
        oa_c[...] = oa
        ds_c[...] = pltpu.bitcast(ds, jnp.uint32)
        dq_c[...] = dq
        return carry

    def pair_body(o, carry):
        g = o // PPG
        first = o % PPG == 0

        @pl.when(jnp.logical_and(first, g > 0))
        def _():
            conv_post(g - 1)

        @pl.when(jnp.logical_and(first, g < NG))
        def _():
            conv_pre(g)

        lax.fori_loop(0, NQ // UNR, lambda j, c2: attn_body(o * (NQ // UNR) + j, c2), 0)
        return carry

    lax.fori_loop(0, NP, pair_body, 0)
    c_dsk.start()
    ddd1[...] = dd_s[1:2, :].reshape(D).astype(bf16)
    c_ddd.start()
    dkq(NIT - 1, 1, NC - 1, pltpu.bitcast(ds_c[...], bf16), dq_c[...])

    def dx_copy(n):
        return cp(wt_s.at[rows_of(n), :], dx_hbm.at[0, rows_of(n), :], SEM_OUT)

    def ob_copy(n):
        return cp(ob_s.at[rows_of(n), :], out_hbm.at[0, rows_of(n), pl.ds(D, D)], SEM_OUT)

    def fin1_body(n, carry):
        cols = rows_of(n)
        db = dqkvt[:, :, cols].reshape(3 * D, XC).astype(bf16)
        dqkvb[:, cols] = db
        oc = dot_s[:, :, cols].reshape(D, XC).T.astype(bf16)
        r = _dg(wqkv_v[...], db, NN)
        wt_s[cols, :] = r.T.astype(bf16)
        ob_s[cols, :] = _dg(oc, wo_v[...], NN).astype(bf16)
        dx_copy(n).start()
        ob_copy(n).start()
        return carry

    lax.fori_loop(0, S // XC, fin1_body, 0)

    def wcols(n):
        return pl.ds(pl.multiple_of(n * 384, 128), 384)

    def dw_copy(n):
        return cp(dwqkv_s.at[:, wcols(n)], dwqkv_hbm.at[:, wcols(n)], SEM_OUT)

    def dwo_copy(n):
        return cp(dwo_s.at[:, lanes_of(n)], dwo_hbm.at[:, lanes_of(n)], SEM_OUT)

    def fin2_body(n, carry):
        dwqkv_s[:, wcols(n)] = _dg(xt_s[...], dqkvb[wcols(n), :], NT).astype(bf16)
        dw_copy(n).start()
        ot = dot_s[...].reshape(D, S)
        dwo_s[:, lanes_of(n)] = _dg(ot, gb_v[:, lanes_of(n)], NN).astype(bf16)
        dwo_copy(n).start()
        return carry

    lax.fori_loop(0, NG, fin2_body, 0)

    for g in range(NG):
        for c in conv_out(g):
            c.wait()
    for n in range(S // XC):
        dx_copy(n).wait()
        ob_copy(n).wait()
    for n in range(NG):
        dw_copy(n).wait()
        dwo_copy(n).wait()
    c_dsk.wait()
    c_ddd.wait()


@jax.jit
def pallas_concat_heads__ssm_conv_h3__softmax_full_mha__prompt_kernel(
    A_q: jax.Array,
    A_k: jax.Array,
    A_v: jax.Array,
    A_shift_k: jax.Array,
    A_ssm_k: jax.Array,
    A_ssm_D: jax.Array,
    B_x: jax.Array,
    B_wqkv: jax.Array,
    B_wo: jax.Array,
    grad_out: jax.Array,
):
    fwd, inv = _dft_mats()
    fwd = jnp.asarray(fwd, dtype=bf16)
    inv = jnp.asarray(inv, dtype=bf16)
    hbm = pl.BlockSpec(memory_space=pl.ANY)
    sd = jax.ShapeDtypeStruct
    V = pltpu.VMEM
    outs = pl.pallas_call(
        _kernel,
        in_specs=[hbm] * 12,
        out_specs=[hbm] * 10,
        out_shape=[
            sd((1, S, 2 * D), bf16), sd((1, S, D), bf16), sd((1, S, D), bf16), sd((1, S, D), bf16),
            sd((4, D), bf16), sd((D, S), bf16), sd((D,), bf16),
            sd((1, S, D), bf16), sd((D, 3 * D), bf16), sd((D, D), bf16),
        ],
        scratch_shapes=[
            V((NG, S, 128), bf16), V((NG, S, 128), bf16), V((NG, S, 128), bf16), V((NG, S, 128), bf16),
            V((D, S), bf16),
            V((S, D), bf16), V((S, D), bf16),
            V((D, 3 * D), bf16), V((D, D), bf16),
            V((S, D), bf16),
            V((3 * NP, G, S), f32),
            V((3 * NP, G, S), f32),
            V((NP, G, S), f32),
            V((NH, S, 128), bf16),
            V((NH, S), f32),
            V((S // 2, TQ), jnp.uint32), V((S // 2, TQ), jnp.uint32),
            V((KS_W, TQ), bf16), V((M, TQ), f32), V((TK // 2, TQ), jnp.uint32), V((M, TQ), f32),
            V((3 * D, S), bf16),
            V((S, D), bf16),
            V((D, S), bf16),
            V((D, 3 * D), bf16), V((D, D), bf16),
            V((S, 128), f32),
            V((3, NPOS, 16 * NB, 128), f32), V((3, NPOS, 16 * NB, 128), f32),
            V((2, NF, CB), bf16), V((2, CB, NF), bf16), V((8, D), f32),
            V((4, D), bf16), V((4, D), bf16), V((D,), bf16), V((D,), bf16),
            pltpu.SemaphoreType.DMA((NSEM,)),
        ],
        compiler_params=pltpu.CompilerParams(vmem_limit_bytes=124 * 1024 * 1024),
        name="h3_mha_fwdbwd",
    )(A_q, A_k, A_v, A_shift_k.T, A_ssm_k, A_ssm_D, B_x, B_wqkv, B_wo, grad_out, fwd, inv)
    out, dq, dk, dv, dsk, dhk, ddd, dx, dwqkv, dwo = outs
    return out, dq, dk, dv, dsk.T, dhk, ddd, dx, dwqkv, dwo
```

```python
import math

import numpy as np
import jax
import jax.numpy as jnp
from jax import lax
import jax.experimental.pallas as pl
import jax.experimental.pallas.tpu as pltpu

f32 = jnp.float32
bf16 = jnp.bfloat16

S = 2048
D = 640
NH = 32
DH = 20
NP = 16
G = 40
M = 24
TQ = 512
TK = 256
NQ = S // TQ
LOG_NQ = NQ.bit_length() - 1
NC = S // TK
NIT = NP * NQ
KS_W = 32
KP_W = 48
R0 = (0, G - M)
V0 = (0, M - DH)
SP0 = (DH, 0)
UNR = 2
CB = 128
NB = S // CB
NF = 2 * CB
NPOS = CB // 8
NG = D // 128
UPG = 3 * NPOS
IPG = UPG // 4
PPG = IPG // NQ
SCALE = DH ** -0.5
LOG2E = math.log2(math.e)
LN2 = math.log(2.0)
SAFE_BOUND = 24.0

NN = (((1,), (0,)), ((), ()))
NT = (((1,), (1,)), ((), ()))

SEM_GB = 0
SEM_W, SEM_X, SEM_CONV, SEM_OUT = 5, 6, 7, 8
NSEM = 9
GB_CHUNKS = ((0, 256), (256, 256), (512, 512), (1024, 512), (1536, 512))


PLAN = tuple(
    (((0, NB - 1 - c),), ((0, c), (1, NB // 2 - 1 - c)), (), (), ((1, NB // 2 + c),), ())
    for c in (2, 0, 3, 6, 4, 5, 1, 7))


def _dg(a, b, dn):
    return lax.dot_general(a, b, dn, preferred_element_type=f32)


def _dft_mats():
    f = np.concatenate([np.arange(0, CB, 2), np.arange(1, CB, 2)]).astype(np.float64)
    n = np.arange(CB, dtype=np.float64)
    th = 2.0 * np.pi * (f[:, None] + 0.5) * n[None, :] / (2 * CB)

    def rows(re, im):
        return np.stack([re.reshape(NPOS, 8, CB), im.reshape(NPOS, 8, CB)], axis=1).reshape(NF, CB)

    fwd = rows(np.cos(th), -np.sin(th))
    fwdc = rows(np.cos(th), np.sin(th))
    fw = np.stack([fwd, fwdc])
    fi = np.stack([fwd.T / CB, fwdc.T / CB])
    return fw.astype(np.float32), fi.astype(np.float32)


def _fill_spare(win, par, b):
    b = -b
    h = b.astype(bf16).astype(f32)
    r = b - h
    m = r.astype(bf16).astype(f32)
    l = (r - m).astype(bf16).astype(f32)
    row = lax.broadcasted_iota(jnp.int32, win.shape, 0)
    s0 = SP0[par]
    return jnp.where(row == s0, h, jnp.where(row == s0 + 1, m, jnp.where(
        row == s0 + 2, l, jnp.where(row == s0 + 3, 0.0, win))))


def _spare_mask(shape, par):
    row = lax.broadcasted_iota(jnp.int32, shape, 0)
    return (row >= DH) if par == 0 else (row < M - DH)


def _shift_add(cur, prev):
    h = NPOS // 2
    cr, ci, pr, pi = cur[:, 0:8], cur[:, 8:16], prev[:, 0:8], prev[:, 8:16]
    re = jnp.concatenate([cr[:h] - pi[:h], cr[h:] + pi[h:]], axis=0)
    im = jnp.concatenate([ci[:h] + pr[:h], ci[h:] - pr[h:]], axis=0)
    return jnp.concatenate([re, im], axis=1)


def _kernel(q_hbm, k_hbm, v_hbm, sk_hbm, hk_hbm, dd_hbm, x_hbm, wqkv_hbm, wo_hbm, g_hbm,
            fw_hbm, fi_hbm,
            out_hbm, dq_hbm, dk_hbm, dv_hbm, dsk_hbm, dhk_hbm, ddd_hbm, dx_hbm, dwqkv_hbm, dwo_hbm,
            q_v, k_v, v_v, ga_v, hk_v, x_v, gb_v, wqkv_v, wo_v,
            wt_s, qkvt, dqkvt, dot_s, kva, b_s, p_a, p_b, qw_c, oa_c, ds_c, dq_c,
            dqkvb, ob_s, xt_s, dwqkv_s, dwo_s,
            ks_s, spec, res, fw_ref, fi_ref, dd_s, sk_ref, dsk_ref, dd1, ddd1,
            sems):
    def cp(src, dst, i):
        return pltpu.make_async_copy(src, dst, sems.at[i])

    XC = 512

    def rows_of(c):
        return pl.ds(pl.multiple_of(c * XC, XC), XC)

    def lanes_of(g):
        return pl.ds(pl.multiple_of(g * 128, 128), 128)

    def conv_in(g):
        return [cp(src.at[0, :, lanes_of(g)], dst.at[g], SEM_CONV)
                for src, dst in ((k_hbm, k_v), (v_hbm, v_v), (q_hbm, q_v), (g_hbm, ga_v))]

    def conv_out(g):
        cs = [cp(src.at[g], dst.at[0, :, lanes_of(g)], SEM_OUT)
              for src, dst in ((k_v, dk_hbm), (v_v, dv_hbm), (q_v, dq_hbm), (ga_v, out_hbm))]
        cs.append(cp(hk_v.at[lanes_of(g), :], dhk_hbm.at[lanes_of(g), :], SEM_OUT))
        return cs

    c_w = cp(wqkv_hbm, wqkv_v, SEM_W)
    c_wo = cp(wo_hbm, wo_v, SEM_GB)
    c_x = cp(x_hbm.at[0], x_v, SEM_X)
    c_gb = [cp(g_hbm.at[0, pl.ds(r0, nr), pl.ds(D, D)], gb_v.at[pl.ds(r0, nr), :], SEM_GB + j)
            for j, (r0, nr) in enumerate(GB_CHUNKS)]
    c_conv = [cp(hk_hbm, hk_v, SEM_CONV), cp(fw_hbm, fw_ref, SEM_CONV), cp(fi_hbm, fi_ref, SEM_CONV),
              cp(sk_hbm, sk_ref, SEM_CONV), cp(dd_hbm, dd1, SEM_CONV)]
    for g in range(NG):
        c_conv += conv_in(g)
    c_dsk = cp(dsk_ref, dsk_hbm, SEM_OUT)
    c_ddd = cp(ddd1, ddd_hbm, SEM_OUT)

    TD = 256
    NDA = 5

    for c in [c_wo] + c_gb[:-1] + [c_w, c_gb[-1], c_x] + c_conv:
        c.start()
    c_wo.wait()
    c_gb[0].wait()

    def dot_chunk(n, waits):
        for j in waits:
            @pl.when(n == GB_CHUNKS[j][0] // TD)
            def _():
                c_gb[j].wait()

        cols = pl.ds(pl.multiple_of(n * TD, TD), TD)
        r = _dg(wo_v[...], gb_v[cols, :], NT)
        dot_s[:, :, cols] = r.reshape(NP, G, TD)

    def dot_body_a(n, carry):
        dot_chunk(n, (1, 2, 3))
        return carry

    def dot_body_b(n, carry):
        dot_chunk(n + NDA, (4,))
        wc = pl.ds(pl.multiple_of(n * D, 128), D)
        wt_s[wc, :] = wqkv_v[:, wc].T
        return carry

    lax.fori_loop(0, NDA, dot_body_a, 0)
    c_w.wait()
    lax.fori_loop(0, S // TD - NDA, dot_body_b, 0)
    c_x.wait()

    def amax8(a):
        return jnp.max(jnp.abs(a).reshape(D // 8, 8, XC), axis=0)

    def proj_body(n, carry):
        cols = rows_of(n)
        xc = x_v[cols, :]
        xt_s[:, cols] = xc.T
        kt = _dg(wt_s[D:2 * D, :], xc, NT)
        qkvt[NP:2 * NP, :, cols] = kt.reshape(NP, G, XC)
        vt = _dg(wt_s[2 * D:3 * D, :], xc, NT)
        qkvt[2 * NP:3 * NP, :, cols] = vt.reshape(NP, G, XC)
        for h in range(NH):
            r0 = (h // 2) * G + R0[h % 2]
            kw = jnp.where(_spare_mask((M, XC), h % 2), 1.0, kt[r0:r0 + M])
            t = jnp.concatenate([kw, vt[r0:r0 + M], jnp.zeros((128 - 2 * M, XC), f32)], axis=0)
            kva[h, cols, :] = t.T.astype(bf16)
        qt = _dg(wt_s[0:D, :], xc, NT) * (SCALE * LOG2E)
        qkvt[0:NP, :, cols] = qt.reshape(NP, G, XC)
        return jnp.maximum(carry[0], amax8(qt)), jnp.maximum(carry[1], amax8(kt))

    qm, km = lax.fori_loop(0, S // XC, proj_body, (jnp.zeros((8, XC), f32), jnp.zeros((8, XC), f32)))

    def allmax(a):
        return jnp.max(jnp.max(a, axis=1, keepdims=True), axis=0, keepdims=True)

    bound = allmax(qm) * allmax(km) * (DH * 1.02)
    b_s[...] = jnp.broadcast_to(bound, b_s.shape)
    unsafe = jnp.logical_not(jnp.max(bound) <= SAFE_BOUND)

    def q_weights(i, par, off, b):
        qt = _fill_spare(qkvt[i, R0[par]:R0[par] + M, pl.ds(off, TQ)], par, b)
        return jnp.concatenate([qt, jnp.zeros((KS_W - M, TQ), f32)], axis=0).astype(bf16)

    @pl.when(unsafe)
    def _():
        def mx_body(t, carry):
            i = t // NQ
            off = pl.multiple_of((t % NQ) * TQ, TQ)
            for par in range(2):
                qw = q_weights(i, par, off, jnp.zeros((1, TQ), f32))

                def mx_chunk(c, m):
                    ro = pl.multiple_of(c * TK, TK)
                    s = _dg(kva[2 * i + par, pl.ds(ro, TK), :KS_W], qw, NN)
                    return jnp.maximum(m, jnp.max(s, axis=0, keepdims=True))

                m = lax.fori_loop(0, NC, mx_chunk, jnp.full((1, TQ), -jnp.inf, f32))
                b_s[pl.ds(2 * i + par, 1), pl.ds(off, TQ)] = m
            return carry
        lax.fori_loop(0, NIT, mx_body, 0)

    for c in c_conv:
        c.wait()
    dd_s[0:1, :] = dd1[...].astype(f32).reshape(1, D)

    def blk(a):
        return slice(16 * a, 16 * a + 16)

    def taps(g):
        w4 = sk_ref[:, lanes_of(g)].astype(f32)
        return [w4[j:j + 1, :] for j in range(4)]

    def conv_pre(g):
        L = lanes_of(g)
        wj = taps(g)
        yp = None
        tail = jnp.zeros((8, 128), f32)
        for a in range(NB):
            r0 = a * CB
            rows = slice(r0, r0 + CB)
            kf = k_v[g, rows, :].astype(f32)
            ext = jnp.concatenate([tail, kf], axis=0)
            tail = kf[CB - 8:CB]
            ks = kf * wj[0]
            for j in range(1, 4):
                ks = ks + pltpu.roll(ext, j, 0)[8:8 + CB] * wj[j]
            ks_s[rows, :] = ks
            kv = ks * v_v[g, rows, :].astype(f32)
            dy = ga_v[g, rows, :].astype(f32) * q_v[g, rows, :].astype(f32)
            h = _dg(fw_ref[0], hk_v[L, rows], NT).reshape(NPOS, 16, 128)
            if a == 0:
                dvec = dd_s[0:1, L]
                h = jnp.concatenate([h[:, 0:8] + dvec[None], h[:, 8:16]], axis=1)
            spec[0, :, blk(a), :] = h
            spec[1, :, blk(a), :] = _dg(fw_ref[0], kv.astype(bf16), NN).reshape(NPOS, 16, 128)
            y = _dg(fw_ref[1], dy.astype(bf16), NN).reshape(NPOS, 16, 128)
            if yp is not None:
                spec[2, :, blk(NB - a), :] = _shift_add(yp, y)
            if a == NB - 1:
                spec[2, :, blk(0), :] = y
            yp = y

    def conv_mac(u):
        u = lax.rem(jnp.minimum(u, NG * UPG - 1), UPG)
        kind = lax.shift_right_logical(u, NPOS.bit_length() - 1)
        pos = u & (NPOS - 1)
        ia = lax.shift_right_logical(kind, 1)
        ib = 1 + jnp.minimum(kind, 1)

        def re(a):
            return slice(16 * a, 16 * a + 8)

        def im(a):
            return slice(16 * a + 8, 16 * a + 16)

        def emit(a):
            zr = zi = None
            for b0 in range(0, a + 1, 4):
                n = min(4, a + 1 - b0)
                av = spec[ia, pos, 16 * b0:16 * (b0 + n), :]
                bv = spec[ib, pos, 16 * (a - b0 - n + 1):16 * (a - b0 + 1), :]
                for j in range(n):
                    ar, ai, br, bi = av[re(j)], av[im(j)], bv[re(n - 1 - j)], bv[im(n - 1 - j)]
                    tr = ar * br - ai * bi
                    ti = ar * bi + ai * br
                    zr = tr if zr is None else zr + tr
                    zi = ti if zi is None else zi + ti
            res[kind, pos, blk(a), :] = jnp.concatenate([zr, zi], axis=0)

        return emit

    def conv_post(g):
        L = lanes_of(g)
        wj = taps(g)
        acc = [jnp.zeros((8, 128), f32) for _ in range(4)]
        head = jnp.zeros((8, 128), f32)
        for a in range(NB - 1, -1, -1):
            r0 = a * CB
            rows = slice(r0, r0 + CB)
            z = res[0, :, blk(a), :]
            if a > 0:
                z = _shift_add(z, res[0, :, blk(a - 1), :])
            dh = _dg(fi_ref[1], res[2, :, blk(NB - 1 - a), :].reshape(NF, 128), NN)
            dkv = _dg(fi_ref[1], res[1, :, blk(NB - 1 - a), :].reshape(NF, 128), NN)
            y = _dg(fi_ref[0], z.reshape(NF, 128), NN)
            hk_v[L, rows] = dh.T.astype(bf16)
            if a == 0:
                dd_s[1:2, L] = dh[0:1, :]
            dks = dkv * v_v[g, rows, :].astype(f32)
            v_v[g, rows, :] = (dkv * ks_s[rows, :]).astype(bf16)
            ext = jnp.concatenate([dks, head], axis=0)
            head = dks[0:8]
            kf = k_v[g, rows, :].astype(f32)
            dk = None
            for j in range(4):
                dj = dks if j == 0 else pltpu.roll(ext, CB + 8 - j, 0)[0:CB]
                dk = dj * wj[j] if dk is None else dk + dj * wj[j]
                acc[j] = acc[j] + jnp.sum((dj * kf).reshape(CB // 8, 8, 128), axis=0)
            k_v[g, rows, :] = dk.astype(bf16)
            qf = q_v[g, rows, :].astype(f32)
            gf = ga_v[g, rows, :].astype(f32)
            ga_v[g, rows, :] = (qf * y).astype(bf16)
            q_v[g, rows, :] = (gf * y).astype(bf16)
        row = lax.broadcasted_iota(jnp.int32, (4, 128), 0)
        r4 = jnp.zeros((4, 128), f32)
        for j in range(4):
            r4 = jnp.where(row == j, jnp.sum(acc[j], axis=0, keepdims=True), r4)
        dsk_ref[:, L] = r4.astype(bf16)
        for c in conv_out(g):
            c.start()

    P = [p_a, p_b]

    def item(t):
        if isinstance(t, int):
            return t // NQ, (t % NQ) * TQ
        return lax.shift_right_logical(t, LOG_NQ), pl.multiple_of((t & (NQ - 1)) * TQ, TQ)

    def make_qw(t, par):
        i, off = item(t)
        return q_weights(i, par, off, b_s[pl.ds(2 * i + par, 1), pl.ds(off, TQ)])

    def finish1(t, par, oa):
        i, off = item(t)
        lo, hi = V0[par], V0[par] + DH
        do = dot_s[i, R0[par]:R0[par] + M, pl.ds(off, TQ)]
        r = 1.0 / oa[SP0[par]:SP0[par] + 1, :]
        o = oa * r
        dop = jnp.where(_spare_mask((M, TQ), par), 0.0, (do * r).astype(bf16).astype(f32))
        dot_s[i, par * DH:(par + 1) * DH, pl.ds(off, TQ)] = o[lo:hi]
        delta = jnp.sum(dop * o, axis=0, keepdims=True)
        top = _fill_spare(jnp.zeros((M, TQ), f32), par, delta)
        return jnp.concatenate([top, dop], axis=0).astype(bf16), dop

    def accum(t, idx, par, ck, val):
        dst = dqkvt.at[idx, par * DH:(par + 1) * DH, ck]
        dst[...] = jnp.where((t & (NQ - 1)) == 0, 0.0, dst[...]) + val

    def dkq(t, par, c, ds, dq, mid=None):
        i, off = item(t)
        lo, hi = V0[par], V0[par] + DH
        ck = slice(c * TK, (c + 1) * TK)
        qt = qkvt[i, R0[par]:R0[par] + M, pl.ds(off, TQ)] * LN2
        dk = _dg(qt, ds, NT)
        accum(t, NP + i, par, ck, dk[lo:hi])
        if mid is not None:
            mid()
        t_ = _dg(qkvt[NP + i, R0[par]:R0[par] + M, ck], ds, NN)
        dq = t_ if dq is None else t_ + dq
        if c == NC - 1:
            dqkvt[i, par * DH:(par + 1) * DH, pl.ds(off, TQ)] = (dq * SCALE)[lo:hi]
        return dq

    def scores(i, par, c, qw):
        s = _dg(kva[2 * i + par, c * TK:(c + 1) * TK, :KS_W], qw, NN)
        p = jnp.exp2(s).astype(bf16)
        P[par][c * TK // 2:(c + 1) * TK // 2, :] = pltpu.bitcast(p, jnp.uint32)
        return p

    def pv(i, par, c, p, oa):
        vt = qkvt[2 * NP + i, R0[par]:R0[par] + M, c * TK:(c + 1) * TK]
        vt = jnp.where(_spare_mask((M, TK), par), 1.0, vt)
        t_ = _dg(vt, p, NN)
        return t_ if oa is None else t_ + oa

    def step(t1, par1, t2, t3, qw, oa2, ds3, dq3, macs):
        par2 = 1 - par1
        i1, _ = item(t1)
        i2, _ = item(t2)
        lo2, hi2 = V0[par2], V0[par2] + DH
        oa = dq = ds = None
        for c in range(NC):
            def fill(slot):
                for k, a in PLAN[c][slot]:
                    macs[k](a)

            ck = slice(c * TK, (c + 1) * TK)
            p1 = scores(i1, par1, c, qw)
            fill(0)
            if c == 0:
                doa, dop = finish1(t2, par2, oa2)
                dkq(t3, par1, NC - 1, ds3, dq3, lambda: fill(1))
            else:
                dq = dkq(t2, par2, c - 1, ds, dq, lambda: fill(1))
            fill(2)
            p2 = pltpu.bitcast(P[par2][c * TK // 2:(c + 1) * TK // 2, :], bf16)
            dp = _dg(kva[2 * i2 + par2, ck, :KP_W], doa, NN)
            ds = (p2.astype(f32) * dp).astype(bf16)
            fill(3)
            dv = _dg(dop, p2, NT)
            accum(t2, 2 * NP + i2, par2, ck, dv[lo2:hi2])
            fill(4)
            oa = pv(i1, par1, c, p1, oa)
            fill(5)
        return oa, ds, dq

    qw0 = make_qw(0, 0)
    oa0 = None
    pprev = None
    for c in range(NC + 1):
        pcur = scores(0, 0, c, qw0) if c < NC else None
        if c > 0:
            oa0 = pv(0, 0, c - 1, pprev, oa0)
        pprev = pcur
    oa_c[...] = oa0
    qw_c[...] = make_qw(0, 1)

    def attn_body(tt, carry):
        @pl.when(tt == 0)
        def _():
            ds_c[...] = jnp.zeros(ds_c.shape, jnp.uint32)
            dq_c[...] = jnp.zeros(dq_c.shape, f32)

        qw_a, oa, dq = qw_c[...], oa_c[...], dq_c[...]
        ds = pltpu.bitcast(ds_c[...], bf16)
        for k in range(UNR):
            t = tt * UNR + k
            tp = jnp.maximum(t - 1, 0)
            tn = jnp.minimum(t + 1, NIT - 1)
            qw_b = make_qw(tn, 0)
            oa, ds, dq = step(t, 1, t, tp, qw_a, oa, ds, dq,
                              [conv_mac(4 * t), conv_mac(4 * t + 1)])
            qw_a = make_qw(tn, 1)
            if k == UNR - 1:
                qw_c[...] = qw_a
            oa, ds, dq = step(tn, 0, t, t, qw_b, oa, ds, dq,
                              [conv_mac(4 * t + 2), conv_mac(4 * t + 3)])
        oa_c[...] = oa
        ds_c[...] = pltpu.bitcast(ds, jnp.uint32)
        dq_c[...] = dq
        return carry

    def pair_body(o, carry):
        g = o // PPG
        first = o % PPG == 0

        @pl.when(jnp.logical_and(first, g > 0))
        def _():
            conv_post(g - 1)

        @pl.when(jnp.logical_and(first, g < NG))
        def _():
            conv_pre(g)

        lax.fori_loop(0, NQ // UNR, lambda j, c2: attn_body(o * (NQ // UNR) + j, c2), 0)
        return carry

    lax.fori_loop(0, NP, pair_body, 0)
    c_dsk.start()
    ddd1[...] = dd_s[1:2, :].reshape(D).astype(bf16)
    c_ddd.start()
    dkq(NIT - 1, 1, NC - 1, pltpu.bitcast(ds_c[...], bf16), dq_c[...])

    def dx_copy(n):
        return cp(wt_s.at[rows_of(n), :], dx_hbm.at[0, rows_of(n), :], SEM_OUT)

    def ob_copy(n):
        return cp(ob_s.at[rows_of(n), :], out_hbm.at[0, rows_of(n), pl.ds(D, D)], SEM_OUT)

    def fin1_body(n, carry):
        cols = rows_of(n)
        db = dqkvt[:, :, cols].reshape(3 * D, XC).astype(bf16)
        dqkvb[:, cols] = db
        oc = dot_s[:, :, cols].reshape(D, XC).T.astype(bf16)
        r = _dg(wqkv_v[...], db, NN)
        wt_s[cols, :] = r.T.astype(bf16)
        ob_s[cols, :] = _dg(oc, wo_v[...], NN).astype(bf16)
        dx_copy(n).start()
        ob_copy(n).start()
        return carry

    lax.fori_loop(0, S // XC, fin1_body, 0)

    def wcols(n):
        return pl.ds(pl.multiple_of(n * 384, 128), 384)

    def dw_copy(n):
        return cp(dwqkv_s.at[:, wcols(n)], dwqkv_hbm.at[:, wcols(n)], SEM_OUT)

    def dwo_copy(n):
        return cp(dwo_s.at[:, lanes_of(n)], dwo_hbm.at[:, lanes_of(n)], SEM_OUT)

    def fin2_body(n, carry):
        dwqkv_s[:, wcols(n)] = _dg(xt_s[...], dqkvb[wcols(n), :], NT).astype(bf16)
        dw_copy(n).start()
        ot = dot_s[...].reshape(D, S)
        dwo_s[:, lanes_of(n)] = _dg(ot, gb_v[:, lanes_of(n)], NN).astype(bf16)
        dwo_copy(n).start()
        return carry

    lax.fori_loop(0, NG, fin2_body, 0)

    for g in range(NG):
        for c in conv_out(g):
            c.wait()
    for n in range(S // XC):
        dx_copy(n).wait()
        ob_copy(n).wait()
    for n in range(NG):
        dw_copy(n).wait()
        dwo_copy(n).wait()
    c_dsk.wait()
    c_ddd.wait()


@jax.jit
def pallas_concat_heads__ssm_conv_h3__softmax_full_mha__prompt_kernel(
    A_q: jax.Array,
    A_k: jax.Array,
    A_v: jax.Array,
    A_shift_k: jax.Array,
    A_ssm_k: jax.Array,
    A_ssm_D: jax.Array,
    B_x: jax.Array,
    B_wqkv: jax.Array,
    B_wo: jax.Array,
    grad_out: jax.Array,
):
    fwd, inv = _dft_mats()
    fwd = jnp.asarray(fwd, dtype=bf16)
    inv = jnp.asarray(inv, dtype=bf16)
    hbm = pl.BlockSpec(memory_space=pl.ANY)
    sd = jax.ShapeDtypeStruct
    V = pltpu.VMEM
    outs = pl.pallas_call(
        _kernel,
        in_specs=[hbm] * 12,
        out_specs=[hbm] * 10,
        out_shape=[
            sd((1, S, 2 * D), bf16), sd((1, S, D), bf16), sd((1, S, D), bf16), sd((1, S, D), bf16),
            sd((4, D), bf16), sd((D, S), bf16), sd((D,), bf16),
            sd((1, S, D), bf16), sd((D, 3 * D), bf16), sd((D, D), bf16),
        ],
        scratch_shapes=[
            V((NG, S, 128), bf16), V((NG, S, 128), bf16), V((NG, S, 128), bf16), V((NG, S, 128), bf16),
            V((D, S), bf16),
            V((S, D), bf16), V((S, D), bf16),
            V((D, 3 * D), bf16), V((D, D), bf16),
            V((S, D), bf16),
            V((3 * NP, G, S), f32),
            V((3 * NP, G, S), f32),
            V((NP, G, S), f32),
            V((NH, S, 128), bf16),
            V((NH, S), f32),
            V((S // 2, TQ), jnp.uint32), V((S // 2, TQ), jnp.uint32),
            V((KS_W, TQ), bf16), V((M, TQ), f32), V((TK // 2, TQ), jnp.uint32), V((M, TQ), f32),
            V((3 * D, S), bf16),
            V((S, D), bf16),
            V((D, S), bf16),
            V((D, 3 * D), bf16), V((D, D), bf16),
            V((S, 128), f32),
            V((3, NPOS, 16 * NB, 128), f32), V((3, NPOS, 16 * NB, 128), f32),
            V((2, NF, CB), bf16), V((2, CB, NF), bf16), V((8, D), f32),
            V((4, D), bf16), V((4, D), bf16), V((D,), bf16), V((D,), bf16),
            pltpu.SemaphoreType.DMA((NSEM,)),
        ],
        compiler_params=pltpu.CompilerParams(vmem_limit_bytes=124 * 1024 * 1024),
        name="h3_mha_fwdbwd",
    )(A_q, A_k, A_v, A_shift_k.T, A_ssm_k, A_ssm_D, B_x, B_wqkv, B_wo, grad_out, fwd, inv)
    out, dq, dk, dv, dsk, dhk, ddd, dx, dwqkv, dwo = outs
    return out, dq, dk, dv, dsk.T, dhk, ddd, dx, dwqkv, dwo
```
